```python
import os as _os
_os.environ.setdefault("JAX_PLATFORMS", "cpu")
import jax
import jax.numpy as jnp

def _softmax(x, axis=-1):
    return jax.nn.softmax(x, axis=axis)
def _gelu(x):
    return jax.nn.gelu(x, approximate=True)
def _silu(x):
    return jax.nn.silu(x)
def _sigmoid(x):
    return jax.nn.sigmoid(x)
def _layernorm(x, axis=-1, eps=1e-5):
    m = jnp.mean(x, axis=axis, keepdims=True)
    v = jnp.var(x, axis=axis, keepdims=True)
    return (x - m) / jnp.sqrt(v + eps)
def _scatter_add(tgt, idx, src, axis=0):
    return tgt.at[idx].add(src)
def _segment_sum(src, seg, n):
    return jax.ops.segment_sum(src, seg, n)
class _Rng:
    def __init__(self, key):
        self._k = key
    def _next(self):
        self._k, sub = jax.random.split(self._k)
        return sub
    def normal(self, shape):
        return jax.random.normal(self._next(), shape, dtype=jnp.bfloat16)
    def randint(self, lo, hi, shape):
        return jax.random.randint(self._next(), shape, lo, hi, dtype=jnp.int32)
    def uniform(self, shape, lo=0.0, hi=1.0):
        return jax.random.uniform(self._next(), shape, jnp.bfloat16, lo, hi)
    def permutation(self, n):
        return jax.random.permutation(self._next(), n)


kernel_name = 'sequential_preLN__mha_block__moe_arch_mod__prompt'

def setup_inputs():
    _rng = _Rng(jax.random.key(int.from_bytes(__import__("os").urandom(4), "little")))
    _w = (lambda a: (lambda t: t.astype(jnp.bfloat16) if jnp.issubdtype(t.dtype, jnp.floating) else t)(jnp.asarray(a)))
    def _A_setup():
        B, S, D, H = 1, 2048, 640, 32
        return {
            "x": _w((lambda *s: _rng.normal(s) * 0.05)(B, S, D)),
            "wqkv": _w((lambda *s: _rng.normal(s) * 0.05)(D, 3 * D)),
            "wo": _w((lambda *s: _rng.normal(s) * 0.05)(D, D)),
        }
    _A_in = _A_setup()

    def _B_setup():
        B, S, D, F, C = 1, 2048, 640, 1536, 1
        return {
            "x": _w((lambda *s: _rng.normal(s) * 0.05)(B, S, D)),
            "w_r": _w((lambda *s: _rng.normal(s) * 0.05)(D)),
            "w_gate": _w((lambda *s: _rng.normal(s) * 0.05)(D, F)),
            "w_up": _w((lambda *s: _rng.normal(s) * 0.05)(D, F)),
            "w_down": _w((lambda *s: _rng.normal(s) * 0.05)(F, D)),
        }
    _B_in = _B_setup()

    return {
        "A_x": _A_in["x"],
        "A_wqkv": _A_in["wqkv"],
        "A_wo": _A_in["wo"],
        "B_x": _B_in["x"],
        "B_w_r": _B_in["w_r"],
        "B_w_gate": _B_in["w_gate"],
        "B_w_up": _B_in["w_up"],
        "B_w_down": _B_in["w_down"],
    }

def reference(A_x, A_wqkv, A_wo, B_x, B_w_r, B_w_gate, B_w_up, B_w_down):
    def _A_ref(x, wqkv, wo):
        B, S, D = x.shape
        H = 32
        Dh = D // H
        qkv = (lambda x, *d: x.transpose(*d))((x @ wqkv).reshape(B, S, 3, H, Dh), 2, 0, 3, 1, 4)
        q, k, v = qkv[0], qkv[1], qkv[2]
        scores = jnp.einsum("bhqd,bhkd->bhqk", q, k) * (Dh ** -0.5)
        p = _softmax(scores, axis=-1)
        o = jnp.einsum("bhqk,bhkd->bhqd", p, v)
        return (lambda x, *d: x.transpose(*d))(o, 0, 2, 1, 3).reshape(B, S, D) @ wo

    def _B_ref(x, w_r, w_gate, w_up, w_down):
        B, S, D = x.shape
        C = 1
        r = x @ w_r
        idx = jnp.argsort(-r, axis=-1)[:, :C]
        idx_e = jnp.repeat(idx.reshape(B, C, 1), D, axis=2)
        x_sel = jnp.take_along_axis(x, idx_e, axis=1)
        g = _silu(x_sel @ w_gate)
        u = x_sel @ w_up
        y = (g * u) @ w_down
        r_sel = _sigmoid(jnp.take_along_axis(r, idx, axis=1))
        y = y * r_sel.reshape(B, C, 1)
        b_off = (jnp.arange(B) * S).reshape(B, 1)
        flat_idx = (idx + b_off).reshape(B * C)
        zero = (x * 0.0).reshape(B * S, D)
        upd = _scatter_add(zero, flat_idx, y.reshape(B * C, D), axis=0)
        return x + upd.reshape(B, S, D)

    x = A_x
    h = x + _A_ref(_layernorm(x, axis=-1), A_wqkv, A_wo)
    h2 = h + _B_ref(_layernorm(h, axis=-1), B_w_r, B_w_gate, B_w_up, B_w_down)
    return h2
```

```python
import functools
import numpy as np
import jax
import jax.numpy as jnp
from jax import lax
import jax.experimental.pallas as pl
import jax.experimental.pallas.tpu as pltpu

S, D, H, DH, F = 2048, 640, 32, 20, 1536
QB = 512
C = 128
NCH = S // C
NQ = S // QB
TP = 256
TW = 256
EPS = 1e-5
QSCALE = float(DH ** -0.5 * np.log2(np.e))
F32 = jnp.float32
BF16 = jnp.bfloat16
NT = (((1,), (1,)), ((), ()))
TN = (((0,), (0,)), ((), ()))
NN = (((1,), (0,)), ((), ()))


def _ln(x):
    mu = jnp.mean(x, axis=-1, keepdims=True)
    d = x - mu
    var = jnp.mean(d * d, axis=-1, keepdims=True)
    return d * lax.rsqrt(var + EPS)


def _kernel(x_hbm, wqkv_hbm, wo_hbm, wr_hbm, wg_hbm, wu_hbm, wd_hbm, out_hbm,
            x_v, wqkv_v, wo_v, wr_v, wg_v, wu_v, wd_v,
            wqT_v, wvT_v, kw_v, qt_v, vt_v, s_v, ot_v, h_v, r_v, ob_v, sems):
    cp_x = pltpu.make_async_copy(x_hbm, x_v, sems.at[0])
    cp_wqkv = pltpu.make_async_copy(wqkv_hbm, wqkv_v, sems.at[1])
    cp_wo = pltpu.make_async_copy(wo_hbm, wo_v, sems.at[2])
    cp_wr = pltpu.make_async_copy(wr_hbm, wr_v, sems.at[3])
    cp_wg = pltpu.make_async_copy(wg_hbm, wg_v, sems.at[4])
    cp_wu = pltpu.make_async_copy(wu_hbm, wu_v, sems.at[5])
    cp_wd = pltpu.make_async_copy(wd_hbm, wd_v, sems.at[6])
    for cp in (cp_x, cp_wqkv, cp_wo, cp_wr, cp_wg, cp_wu, cp_wd):
        cp.start()
    cp_wqkv.wait()
    wqT_v[...] = wqkv_v[:, 0:D].T
    wvT_v[...] = wqkv_v[:, 2 * D:3 * D].T
    cp_x.wait()

    def proj_body(c, carry):
        r0 = pl.multiple_of(c * TP, TP)
        x = x_v[pl.ds(r0, TP), :].astype(F32)
        xn = _ln(x).astype(BF16)
        k = jnp.dot(xn, wqkv_v[:, D:2 * D], preferred_element_type=F32).astype(BF16)
        for w in range(5):
            kw_v[w, pl.ds(r0, TP), :] = k[:, 128 * w:128 * (w + 1)]
        for j in range(4):
            kw_v[5 + j, pl.ds(r0, TP), :] = k[:, 64 + 128 * j:192 + 128 * j]
        qt = lax.dot_general(wqT_v[...], xn, NT, preferred_element_type=F32)
        qt_v[:, pl.ds(r0, TP)] = (qt * QSCALE).astype(BF16)
        vt = lax.dot_general(wvT_v[...], xn, NT, preferred_element_type=F32)
        vt_v[:, pl.ds(r0, TP)] = vt.astype(BF16).astype(F32)
        return carry

    lax.fori_loop(0, S // TP, proj_body, 0)

    def head_geom(h):
        f0 = h * DH
        t = f0 // 128
        rem = f0 - t * 128
        strad = rem > 128 - DH
        win = jnp.where(strad, 5 + t, t)
        o = t * 128 + jnp.where(strad, 64, 0)
        return win, pl.multiple_of(o, 64), f0 - o

    def getq(h, qb):
        h = jnp.minimum(h, H - 1)
        win, o, lo = head_geom(h)
        qt = qt_v[pl.ds(o, 128), qb * QB:(qb + 1) * QB]
        rows = lax.broadcasted_iota(jnp.int32, (128, QB), 0)
        qt = jnp.where((rows >= lo) & (rows < lo + DH), qt.astype(F32), 0.0).astype(BF16)
        return win, qt

    def stageA(A, half, j, mx):
        win, qt = A
        kk = kw_v[win, j * C:(j + 1) * C, :]
        s = jnp.dot(kk, qt, preferred_element_type=F32)
        s_v[half * S + j * C:half * S + (j + 1) * C, :] = s
        mj = jnp.max(s.reshape(C // 8, 8, QB), axis=0)
        return mj if mx is None else jnp.maximum(mx, mj)

    def stageB(a_h, ones_mask, half, j, m, acc):
        s = s_v[half * S + j * C:half * S + (j + 1) * C, :]
        p = jnp.exp2(s - m).astype(BF16)
        vt = vt_v[pl.ds(a_h, 24), j * C:(j + 1) * C]
        vt = jnp.where(ones_mask, 1.0, vt)
        pv = lax.dot_general(vt, p, NN, preferred_element_type=F32)
        return pv if acc is None else acc + pv

    def red(mx):
        return jnp.max(mx, axis=0, keepdims=True)

    A0 = getq(0, 0)
    mx = None
    for j in range(NCH):
        mx = stageA(A0, 0, j, mx)
    m0 = red(mx)
    mx1 = stageA(getq(0, 1), 1, 0, None)

    def head_body(h, carry):
        m, mxn = carry
        odd = (h % 2) == 1
        a_h = pl.multiple_of(h * DH - (h % 2) * 4, 8)
        row24 = lax.broadcasted_iota(jnp.int32, (24, C), 0)
        ones_mask = row24 == jnp.where(odd, 0, 20)
        row24q = lax.broadcasted_iota(jnp.int32, (24, QB), 0)
        lo_v = jnp.where(odd, 4, 0)
        valid = (row24q >= lo_v) & (row24q < lo_v + DH)

        def item(u):
            return getq(h + u // NQ, u % NQ)

        An = item(1)
        for u in range(NQ):
            Anext = item(u + 2)
            acc = None
            mx2 = None
            for c in range(NCH):
                if c + 1 < NCH:
                    mxn = stageA(An, (u + 1) % 2, c + 1, mxn)
                else:
                    mx2 = stageA(Anext, u % 2, 0, mx2)
                acc = stageB(a_h, ones_mask, u % 2, c, m, acc)
            l = jnp.where(odd, acc[0:1, :], acc[20:21, :])
            o = acc * (1.0 / l)
            pltpu.store(ot_v.at[pl.ds(a_h, 24), u * QB:(u + 1) * QB], o, mask=valid)
            m = red(mxn)
            mxn = mx2
            An = Anext
        return m, mxn

    lax.fori_loop(0, H, head_body, (m0, mx1))

    cp_wo.wait()
    cp_wr.wait()
    wr = wr_v[...].astype(F32).reshape(1, D)

    def out_body(c, carry):
        r0 = pl.multiple_of(c * TW, TW)
        ot = ot_v[:, pl.ds(r0, TW)].astype(BF16)
        attn = lax.dot_general(ot, wo_v[...], TN, preferred_element_type=F32)
        h = x_v[pl.ds(r0, TW), :].astype(F32) + attn
        h_v[pl.ds(r0, TW), :] = h
        hn = _ln(h)
        ob_v[pl.ds(r0, TW), :] = (h + hn).astype(BF16)
        hb = hn.astype(BF16).astype(F32)
        r_v[pl.ds(r0, TW), :] = jnp.sum(hb * wr, axis=-1, keepdims=True)
        return carry

    lax.fori_loop(0, S // TW, out_body, 0)

    r = r_v[...]
    rmax = jnp.max(r)
    tok = lax.broadcasted_iota(jnp.int32, (S, 1), 0)
    idx = jnp.min(jnp.where(r == rmax, tok, S - 1))
    g0 = pl.multiple_of((idx // 16) * 16, 16)
    hg = h_v[pl.ds(g0, 16), :]
    hng = _ln(hg)
    xs = hng.astype(BF16)
    cp_wg.wait()
    cp_wu.wait()
    cp_wd.wait()
    a = jnp.dot(xs, wg_v[...], preferred_element_type=F32)
    u = jnp.dot(xs, wu_v[...], preferred_element_type=F32)
    a = a.astype(BF16).astype(F32)
    u = u.astype(BF16).astype(F32)
    gu = (a * jax.nn.sigmoid(a) * u).astype(BF16)
    y = jnp.dot(gu, wd_v[...], preferred_element_type=F32)
    rs = jax.nn.sigmoid(jnp.full((1, 1), rmax, F32))
    sel = lax.broadcasted_iota(jnp.int32, (16, D), 0) == (idx - g0)
    ob_v[pl.ds(g0, 16), :] = (hg + hng + jnp.where(sel, y * rs, 0.0)).astype(BF16)
    cp_o = pltpu.make_async_copy(ob_v, out_hbm, sems.at[7])
    cp_o.start()
    cp_o.wait()


@jax.jit
def pallas_sequential_preLN__mha_block__moe_arch_mod__prompt_kernel(
        A_x, A_wqkv, A_wo, B_x, B_w_r, B_w_gate, B_w_up, B_w_down):
    del B_x
    x = A_x.reshape(S, D)
    anyspec = pl.BlockSpec(memory_space=pl.ANY)
    out = pl.pallas_call(
        _kernel,
        out_shape=jax.ShapeDtypeStruct((S, D), BF16),
        in_specs=[anyspec] * 7,
        out_specs=anyspec,
        scratch_shapes=[
            pltpu.VMEM((S, D), BF16), pltpu.VMEM((D, 3 * D), BF16), pltpu.VMEM((D, D), BF16),
            pltpu.VMEM((D,), BF16), pltpu.VMEM((D, F), BF16), pltpu.VMEM((D, F), BF16),
            pltpu.VMEM((F, D), BF16),
            pltpu.VMEM((D, D), BF16), pltpu.VMEM((D, D), BF16),
            pltpu.VMEM((9, S, 128), BF16), pltpu.VMEM((D, S), BF16), pltpu.VMEM((D, S), F32),
            pltpu.VMEM((2 * S, QB), F32), pltpu.VMEM((D, S), F32), pltpu.VMEM((S, D), F32),
            pltpu.VMEM((S, 1), F32), pltpu.VMEM((S, D), BF16),
            pltpu.SemaphoreType.DMA((8,)),
        ],
        compiler_params=pltpu.CompilerParams(vmem_limit_bytes=100 * 1024 * 1024),
        name="seqk",
    )(x, A_wqkv, A_wo, B_w_r, B_w_gate, B_w_up, B_w_down)
    return out.reshape(1, S, D)
```

```python
import functools
import numpy as np
import jax
import jax.numpy as jnp
from jax import lax
import jax.experimental.pallas as pl
import jax.experimental.pallas.tpu as pltpu

S, D, H, DH, F = 2048, 640, 32, 20, 1536
QB = 512
C = 128
NCH = S // C
NQ = S // QB
TP = 256
NP = S // TP
TW = 128
NW = S // TW
TO = 256
NO = S // TO
HPB = 2
PEEL = 2
EPS = 1e-5
QSCALE = float(DH ** -0.5 * np.log2(np.e))
F32 = jnp.float32
BF16 = jnp.bfloat16
NT = (((1,), (1,)), ((), ()))
TN = (((0,), (0,)), ((), ()))
NN = (((1,), (0,)), ((), ()))


def _ln(x):
    mu = jnp.mean(x, axis=-1, keepdims=True)
    d = x - mu
    var = jnp.mean(d * d, axis=-1, keepdims=True)
    return d * lax.rsqrt(var + EPS)


def _kernel(x_hbm, wqkv_hbm, wo_hbm, wr_hbm, wg_hbm, wu_hbm, wd_hbm, out_hbm,
            x_v, wq_v, wk_v, wv_v, wo_v, wr_v, wg_v, wu_v, wd_v,
            xn_v, kw_v, qt_v, vt_v, s_v, ot_v, h_v, hn_v, ob_v, fx_v,
            xsem, wsem, osem):
    def xcopy(r0, n, i):
        return pltpu.make_async_copy(x_hbm.at[pl.ds(r0, n)], x_v.at[pl.ds(r0, n)], xsem.at[i])
    cp_x0 = xcopy(0, TP, 0)
    cp_x1 = xcopy(TP, TP, 1)
    cp_x2 = xcopy(2 * TP, S - 2 * TP, 2)
    cp_wq = pltpu.make_async_copy(wqkv_hbm.at[:, pl.ds(0, D)], wq_v, wsem.at[0])
    cp_wk = pltpu.make_async_copy(wqkv_hbm.at[:, pl.ds(D, D)], wk_v, wsem.at[1])
    cp_wv = pltpu.make_async_copy(wqkv_hbm.at[:, pl.ds(2 * D, D)], wv_v, wsem.at[2])
    cp_wo = pltpu.make_async_copy(wo_hbm, wo_v, wsem.at[3])
    cp_wr = pltpu.make_async_copy(wr_hbm, wr_v, wsem.at[4])
    cp_wg = pltpu.make_async_copy(wg_hbm, wg_v, wsem.at[5])
    cp_wu = pltpu.make_async_copy(wu_hbm, wu_v, wsem.at[6])
    cp_wd = pltpu.make_async_copy(wd_hbm, wd_v, wsem.at[7])
    for cp in (cp_x0, cp_wk, cp_x1):
        cp.start()

    def ln1(r0, n):
        xn_v[r0:r0 + n, :] = _ln(x_v[r0:r0 + n, :].astype(F32)).astype(BF16)

    def kproj(c):
        r0 = c * TP
        k = jnp.dot(xn_v[r0:r0 + TP, :], wk_v[...], preferred_element_type=F32).astype(BF16)
        for w in range(5):
            kw_v[w, r0:r0 + TP, :] = k[:, 128 * w:128 * (w + 1)]
        for j in range(4):
            kw_v[5 + j, r0:r0 + TP, :] = k[:, 64 + 128 * j:192 + 128 * j]

    def qproj(c):
        r0 = c * TP
        q = jnp.dot(xn_v[r0:r0 + TP, :], wq_v[...], preferred_element_type=F32)
        qt_v[:, r0:r0 + TP] = (q * QSCALE).astype(BF16).T

    def vproj(c):
        r0 = c * TP
        v = jnp.dot(xn_v[r0:r0 + TP, :], wv_v[...], preferred_element_type=F32)
        vt_v[:, r0:r0 + TP] = v.astype(BF16).T.astype(F32)

    cp_x0.wait()
    cp_wq.start()
    cp_wv.start()
    ln1(0, TP)
    cp_wk.wait()
    cp_x1.wait()
    cp_x2.start()
    kproj(0)
    ln1(TP, TP)
    kproj(1)
    cp_wq.wait()
    cp_wv.wait()
    for cp in (cp_wo, cp_wr, cp_wg, cp_wu, cp_wd):
        cp.start()
    qproj(0)
    vproj(0)
    cp_x2.wait()
    qproj(1)
    ln1(2 * TP, TP // 2)
    vproj(1)
    ln1(2 * TP + TP // 2, TP // 2)
    for c in range(2, NP):
        qproj(c)
        if c + 1 < NP:
            ln1((c + 1) * TP, TP // 2)
        kproj(c)
        if c + 1 < NP:
            ln1((c + 1) * TP + TP // 2, TP // 2)
        vproj(c)

    def head_geom(h):
        f0 = h * DH
        t = f0 // 128
        rem = f0 - t * 128
        if isinstance(h, int):
            strad = rem > 128 - DH
            win = 5 + t if strad else t
            o = t * 128 + (64 if strad else 0)
            return win, o, f0 - o
        strad = rem > 128 - DH
        win = jnp.where(strad, 5 + t, t)
        o = t * 128 + jnp.where(strad, 64, 0)
        return win, pl.multiple_of(o, 64), f0 - o

    def getq(h, qb):
        win, o, lo = head_geom(h)
        qt = qt_v[pl.ds(o, 128), qb * QB:(qb + 1) * QB]
        rows = lax.broadcasted_iota(jnp.int32, (128, QB), 0)
        qt = jnp.where((rows >= lo) & (rows < lo + DH), qt.astype(F32), 0.0).astype(BF16)
        return win, qt

    def stageA(A, half, j, mx):
        win, qt = A
        kk = kw_v[win, j * C:(j + 1) * C, :]
        s = jnp.dot(kk, qt, preferred_element_type=F32)
        s_v[half * S + j * C:half * S + (j + 1) * C, :] = s
        mj = jnp.max(s.reshape(C // 8, 8, QB), axis=0)
        return mj if mx is None else jnp.maximum(mx, mj)

    def stageB(a_h, ones_mask, half, j, m, acc):
        s = s_v[half * S + j * C:half * S + (j + 1) * C, :]
        p = jnp.exp2(s - m).astype(BF16)
        vt = vt_v[pl.ds(a_h, 24), j * C:(j + 1) * C]
        vt = jnp.where(ones_mask, 1.0, vt)
        pv = lax.dot_general(vt, p, NN, preferred_element_type=F32)
        return pv if acc is None else acc + pv

    def red(mx):
        return jnp.max(mx, axis=0, keepdims=True)

    A0 = getq(0, 0)
    mx = None
    for j in range(NCH):
        mx = stageA(A0, 0, j, mx)
    m0 = red(mx)
    mx1 = stageA(getq(0, 1), 1, 0, None)

    def heads(h0, nh, carry, last, filler=None):
        m, mxn = carry
        nit = nh * NQ

        def item(u):
            if last and u >= nit:
                return None
            return getq(h0 + u // NQ, u % NQ)

        An = item(1)
        for hh in range(nh):
            h = h0 + hh
            odd = (hh % 2) == 1
            a_h = h * DH - (hh % 2) * 4
            if not isinstance(a_h, int):
                a_h = pl.multiple_of(a_h, 8)
            lo_v = 4 if odd else 0
            ones_row = 0 if odd else 20
            row24 = lax.broadcasted_iota(jnp.int32, (24, C), 0)
            ones_mask = row24 == ones_row
            row24q = lax.broadcasted_iota(jnp.int32, (24, QB), 0)
            valid = (row24q >= lo_v) & (row24q < lo_v + DH)
            for uu in range(NQ):
                u = hh * NQ + uu
                Anext = item(u + 2)
                acc = None
                mx2 = None
                for c in range(NCH):
                    if c + 1 < NCH:
                        if An is not None:
                            mxn = stageA(An, (u + 1) % 2, c + 1, mxn)
                    elif Anext is not None:
                        mx2 = stageA(Anext, u % 2, 0, mx2)
                    acc = stageB(a_h, ones_mask, u % 2, c, m, acc)
                    if filler is not None:
                        filler(u, c)
                l = acc[0:1, :] if odd else acc[20:21, :]
                o = acc * (1.0 / l)
                pltpu.store(ot_v.at[pl.ds(a_h, 24), uu * QB:(uu + 1) * QB], o, mask=valid)
                if An is not None:
                    m = red(mxn)
                mxn = mx2
                An = Anext
        return m, mxn

    carry = lax.fori_loop(0, (H - PEEL) // HPB, lambda hb, cr: heads(hb * HPB, HPB, cr, False), (m0, mx1))

    cp_o = [pltpu.make_async_copy(ob_v.at[pl.ds(c * TO, TO)], out_hbm.at[pl.ds(c * TO, TO)], osem.at[c])
            for c in range(NO)]
    st = {}

    def wM(c):
        r0 = c * TW
        ot = ot_v[:, r0:r0 + TW].astype(BF16)
        attn = lax.dot_general(ot, wo_v[...], TN, preferred_element_type=F32)
        h_v[r0:r0 + TW, :] = x_v[r0:r0 + TW, :].astype(F32) + attn

    def wL(c):
        r0 = c * TW
        h = h_v[r0:r0 + TW, :]
        hn = _ln(h)
        ob_v[r0:r0 + TW, :] = (h + hn).astype(BF16)
        if (r0 + TW) % TO == 0:
            cp_o[r0 // TO].start()
        hn_v[r0:r0 + TW, :] = hn.astype(BF16)
        r = jnp.sum(hn * st['wr'], axis=-1, keepdims=True)
        r3 = r.reshape(TW // 8, 8, 1)
        tok = r0 + lax.broadcasted_iota(jnp.int32, (TW // 8, 8, 1), 0) * 8 \
            + lax.broadcasted_iota(jnp.int32, (TW // 8, 8, 1), 1)
        cmax = jnp.max(r3, axis=0)
        cidx = jnp.min(jnp.where(r3 == cmax[None], tok, S), axis=0)
        if 'best' not in st:
            st['best'], st['bidx'] = cmax, cidx
        else:
            gt = cmax > st['best']
            st['best'] = jnp.where(gt, cmax, st['best'])
            st['bidx'] = jnp.where(gt, cidx, st['bidx'])

    NFILL = 4

    def filler(u, c):
        if u == PEEL * NQ - 1 and c % (NCH // NFILL) == 1:
            wM(c // (NCH // NFILL))

    cp_wo.wait()
    cp_wr.wait()
    st['wr'] = wr_v[...].astype(F32).reshape(1, D)
    heads(H - PEEL, PEEL, carry, True, filler)
    LAG = 1
    for c in range(NW + LAG):
        if NFILL <= c + NFILL - LAG < NW and c + NFILL - LAG >= NFILL:
            wM(c + NFILL - LAG)
        if c >= LAG:
            wL(c - LAG)
    best, bidx = st['best'], st['bidx']

    rmax = jnp.max(best)
    idx = jnp.min(jnp.where(best == rmax, bidx, S - 1))
    idx = jnp.minimum(idx, S - 1)
    g0 = pl.multiple_of((idx // 16) * 16, 16)
    xs = hn_v[pl.ds(g0, 16), :]
    cp_wg.wait()
    cp_wu.wait()
    cp_wd.wait()
    a = jnp.dot(xs, wg_v[...], preferred_element_type=F32)
    u = jnp.dot(xs, wu_v[...], preferred_element_type=F32)
    a = a.astype(BF16).astype(F32)
    u = u.astype(BF16).astype(F32)
    gu = (a * jax.nn.sigmoid(a) * u).astype(BF16)
    y = jnp.dot(gu, wd_v[...], preferred_element_type=F32)
    rs = jax.nn.sigmoid(jnp.full((1, 1), rmax, F32))
    sel = lax.broadcasted_iota(jnp.int32, (16, D), 0) == (idx - g0)
    base = ob_v[pl.ds(g0, 16), :].astype(F32)
    fx_v[...] = (base + jnp.where(sel, y * rs, 0.0)).astype(BF16)
    for c in range(NO):
        cp_o[c].wait()
    cp_f = pltpu.make_async_copy(fx_v, out_hbm.at[pl.ds(g0, 16)], osem.at[NO])
    cp_f.start()
    cp_f.wait()


@jax.jit
def pallas_sequential_preLN__mha_block__moe_arch_mod__prompt_kernel(
        A_x, A_wqkv, A_wo, B_x, B_w_r, B_w_gate, B_w_up, B_w_down):
    del B_x
    x = A_x.reshape(S, D)
    anyspec = pl.BlockSpec(memory_space=pl.ANY)
    out = pl.pallas_call(
        _kernel,
        out_shape=jax.ShapeDtypeStruct((S, D), BF16),
        in_specs=[anyspec] * 7,
        out_specs=anyspec,
        scratch_shapes=[
            pltpu.VMEM((S, D), BF16), pltpu.VMEM((D, D), BF16), pltpu.VMEM((D, D), BF16),
            pltpu.VMEM((D, D), BF16), pltpu.VMEM((D, D), BF16),
            pltpu.VMEM((D,), BF16), pltpu.VMEM((D, F), BF16), pltpu.VMEM((D, F), BF16),
            pltpu.VMEM((F, D), BF16),
            pltpu.VMEM((S, D), BF16),
            pltpu.VMEM((9, S, 128), BF16), pltpu.VMEM((D, S), BF16), pltpu.VMEM((D, S), F32),
            pltpu.VMEM((2 * S, QB), F32), pltpu.VMEM((D, S), F32), pltpu.VMEM((S, D), F32),
            pltpu.VMEM((S, D), BF16),
            pltpu.VMEM((S, D), BF16), pltpu.VMEM((16, D), BF16),
            pltpu.SemaphoreType.DMA((3,)), pltpu.SemaphoreType.DMA((8,)),
            pltpu.SemaphoreType.DMA((NO + 1,)),
        ],
        compiler_params=pltpu.CompilerParams(vmem_limit_bytes=100 * 1024 * 1024),
        name="seqk",
    )(x, A_wqkv, A_wo, B_w_r, B_w_gate, B_w_up, B_w_down)
    return out.reshape(1, S, D)
```

```python
import numpy as np
import jax
import jax.numpy as jnp
from jax import lax
import jax.experimental.pallas as pl
import jax.experimental.pallas.tpu as pltpu

S, D, H, DH, F = 2048, 640, 32, 20, 1536
QB = 512
C = 128
NCH = S // C
NQ = S // QB
TP = 256
NP = S // TP
TW = 128
NW = S // TW
TO = 256
NO = S // TO
HPB = 2
PEEL = 2
NFILL = 4
EPS = 1e-5
QSCALE = float(DH ** -0.5 * np.log2(np.e))
F32 = jnp.float32
BF16 = jnp.bfloat16
TN = (((0,), (0,)), ((), ()))
NN = (((1,), (0,)), ((), ()))


def _ln(x):
    mu = jnp.mean(x, axis=-1, keepdims=True)
    d = x - mu
    var = jnp.mean(d * d, axis=-1, keepdims=True)
    return d * lax.rsqrt(var + EPS)


def _kernel(x_hbm, wqkv_hbm, wo_hbm, wr_hbm, wg_hbm, wu_hbm, wd_hbm, out_hbm,
            x_v, wq_v, wk_v, wv_v, wo_v, wr_v, wg_v, wu_v, wd_v,
            xn_v, kw_v, qt_v, vt_v, s_v, ot_v, h_v, hn_v, ob_v, fx_v,
            xsem, wsem, osem):
    def xcopy(r0, n, i):
        return pltpu.make_async_copy(x_hbm.at[pl.ds(r0, n)], x_v.at[pl.ds(r0, n)], xsem.at[i])
    cp_x0 = xcopy(0, TP, 0)
    cp_x1 = xcopy(TP, TP, 1)
    cp_x2 = xcopy(2 * TP, S - 2 * TP, 2)
    cp_wq = pltpu.make_async_copy(wqkv_hbm.at[:, pl.ds(0, D)], wq_v, wsem.at[0])
    cp_wk = pltpu.make_async_copy(wqkv_hbm.at[:, pl.ds(D, D)], wk_v, wsem.at[1])
    cp_wv = pltpu.make_async_copy(wqkv_hbm.at[:, pl.ds(2 * D, D)], wv_v, wsem.at[2])
    cp_wo = pltpu.make_async_copy(wo_hbm, wo_v, wsem.at[3])
    cp_wr = pltpu.make_async_copy(wr_hbm, wr_v, wsem.at[4])
    cp_wg = pltpu.make_async_copy(wg_hbm, wg_v, wsem.at[5])
    cp_wu = pltpu.make_async_copy(wu_hbm, wu_v, wsem.at[6])
    cp_wd = pltpu.make_async_copy(wd_hbm, wd_v, wsem.at[7])
    for cp in (cp_x0, cp_wk, cp_x1):
        cp.start()

    def ln1(r0, n):
        xn_v[r0:r0 + n, :] = _ln(x_v[r0:r0 + n, :].astype(F32)).astype(BF16)

    def kproj(c):
        r0 = c * TP
        k = jnp.dot(xn_v[r0:r0 + TP, :], wk_v[...], preferred_element_type=F32).astype(BF16)
        for w in range(5):
            kw_v[w, r0:r0 + TP, :] = k[:, 128 * w:128 * (w + 1)]
        for j in range(4):
            kw_v[5 + j, r0:r0 + TP, :] = k[:, 64 + 128 * j:192 + 128 * j]

    def qproj(c):
        r0 = c * TP
        q = jnp.dot(xn_v[r0:r0 + TP, :], wq_v[...], preferred_element_type=F32)
        qt_v[:, r0:r0 + TP] = (q * QSCALE).astype(BF16).T

    def vproj(c):
        r0 = c * TP
        v = jnp.dot(xn_v[r0:r0 + TP, :], wv_v[...], preferred_element_type=F32)
        vt_v[:, r0:r0 + TP] = v.astype(BF16).T.astype(F32)

    cp_x0.wait()
    cp_wq.start()
    cp_wv.start()
    ln1(0, TP)
    cp_wk.wait()
    cp_x1.wait()
    cp_x2.start()
    kproj(0)
    ln1(TP, TP)
    kproj(1)
    cp_wq.wait()
    cp_wv.wait()
    for cp in (cp_wo, cp_wr, cp_wg, cp_wu, cp_wd):
        cp.start()
    qproj(0)
    vproj(0)
    cp_x2.wait()
    qproj(1)
    ln1(2 * TP, TP // 2)
    vproj(1)
    ln1(2 * TP + TP // 2, TP // 2)
    for c in range(2, NP):
        qproj(c)
        if c + 1 < NP:
            ln1((c + 1) * TP, TP // 2)
        kproj(c)
        if c + 1 < NP:
            ln1((c + 1) * TP + TP // 2, TP // 2)
        vproj(c)

    def head_geom(h):
        f0 = h * DH
        t = f0 // 128
        rem = f0 - t * 128
        strad = rem > 128 - DH
        if isinstance(h, int):
            o = t * 128 + (64 if strad else 0)
            return (5 + t if strad else t), o, f0 - o
        win = jnp.where(strad, 5 + t, t)
        o = t * 128 + jnp.where(strad, 64, 0)
        return win, pl.multiple_of(o, 64), f0 - o

    def getq(h, qb):
        win, o, lo = head_geom(h)
        qt = qt_v[pl.ds(o, 128), qb * QB:(qb + 1) * QB]
        rows = lax.broadcasted_iota(jnp.int32, (128, QB), 0)
        qt = jnp.where((rows >= lo) & (rows < lo + DH), qt.astype(F32), 0.0).astype(BF16)
        return win, qt

    def stage_a(item, half, j, mx):
        win, qt = item
        s = jnp.dot(kw_v[win, j * C:(j + 1) * C, :], qt, preferred_element_type=F32)
        s_v[half * S + j * C:half * S + (j + 1) * C, :] = s
        mj = jnp.max(s.reshape(C // 8, 8, QB), axis=0)
        return mj if mx is None else jnp.maximum(mx, mj)

    def stage_b(a_h, ones_mask, half, j, m, acc):
        s = s_v[half * S + j * C:half * S + (j + 1) * C, :]
        p = jnp.exp2(s - m).astype(BF16)
        vt = vt_v[pl.ds(a_h, 24), j * C:(j + 1) * C]
        vt = jnp.where(ones_mask, 1.0, vt)
        pv = lax.dot_general(vt, p, NN, preferred_element_type=F32)
        return pv if acc is None else acc + pv

    def red(mx):
        return jnp.max(mx, axis=0, keepdims=True)

    item0 = getq(0, 0)
    mx = None
    for j in range(NCH):
        mx = stage_a(item0, 0, j, mx)
    m0 = red(mx)
    mx1 = stage_a(getq(0, 1), 1, 0, None)

    def heads(h0, nh, carry, last, filler=None):
        m, mxn = carry
        nit = nh * NQ

        def item(u):
            if last and u >= nit:
                return None
            return getq(h0 + u // NQ, u % NQ)

        nxt = item(1)
        for hh in range(nh):
            h = h0 + hh
            odd = (hh % 2) == 1
            a_h = h * DH - (hh % 2) * 4
            if not isinstance(a_h, int):
                a_h = pl.multiple_of(a_h, 8)
            lo_v = 4 if odd else 0
            ones_row = 0 if odd else 20
            ones_mask = lax.broadcasted_iota(jnp.int32, (24, C), 0) == ones_row
            row24q = lax.broadcasted_iota(jnp.int32, (24, QB), 0)
            valid = (row24q >= lo_v) & (row24q < lo_v + DH)
            for uu in range(NQ):
                u = hh * NQ + uu
                nxt2 = item(u + 2)
                acc = None
                mx2 = None
                for c in range(NCH):
                    if c + 1 < NCH:
                        if nxt is not None:
                            mxn = stage_a(nxt, (u + 1) % 2, c + 1, mxn)
                    elif nxt2 is not None:
                        mx2 = stage_a(nxt2, u % 2, 0, mx2)
                    acc = stage_b(a_h, ones_mask, u % 2, c, m, acc)
                    if filler is not None:
                        filler(u, c)
                denom = acc[ones_row:ones_row + 1, :]
                o = acc * (1.0 / denom)
                pltpu.store(ot_v.at[pl.ds(a_h, 24), uu * QB:(uu + 1) * QB], o, mask=valid)
                if nxt is not None:
                    m = red(mxn)
                mxn = mx2
                nxt = nxt2
        return m, mxn

    carry = lax.fori_loop(0, (H - PEEL) // HPB,
                          lambda hb, cr: heads(hb * HPB, HPB, cr, False), (m0, mx1))

    cp_o = [pltpu.make_async_copy(ob_v.at[pl.ds(c * TO, TO)], out_hbm.at[pl.ds(c * TO, TO)], osem.at[c])
            for c in range(NO)]
    st = {}

    def w_proj(c):
        r0 = c * TW
        ot = ot_v[:, r0:r0 + TW].astype(BF16)
        attn = lax.dot_general(ot, wo_v[...], TN, preferred_element_type=F32)
        h_v[r0:r0 + TW, :] = x_v[r0:r0 + TW, :].astype(F32) + attn

    def w_norm(c):
        r0 = c * TW
        h = h_v[r0:r0 + TW, :]
        hn = _ln(h)
        ob_v[r0:r0 + TW, :] = (h + hn).astype(BF16)
        if (r0 + TW) % TO == 0:
            cp_o[r0 // TO].start()
        hn_v[r0:r0 + TW, :] = hn.astype(BF16)
        r = jnp.sum(hn * st['wr'], axis=-1, keepdims=True)
        r3 = r.reshape(TW // 8, 8, 1)
        tok = r0 + lax.broadcasted_iota(jnp.int32, (TW // 8, 8, 1), 0) * 8 \
            + lax.broadcasted_iota(jnp.int32, (TW // 8, 8, 1), 1)
        cmax = jnp.max(r3, axis=0)
        cidx = jnp.min(jnp.where(r3 == cmax[None], tok, S), axis=0)
        if 'best' not in st:
            st['best'], st['bidx'] = cmax, cidx
        else:
            gt = cmax > st['best']
            st['best'] = jnp.where(gt, cmax, st['best'])
            st['bidx'] = jnp.where(gt, cidx, st['bidx'])

    def filler(u, c):
        if u == PEEL * NQ - 1 and c % (NCH // NFILL) == 1:
            w_proj(c // (NCH // NFILL))

    cp_wo.wait()
    cp_wr.wait()
    st['wr'] = wr_v[...].astype(F32).reshape(1, D)
    heads(H - PEEL, PEEL, carry, True, filler)
    for c in range(NW + 1):
        if 1 <= c and c + NFILL - 1 < NW:
            w_proj(c + NFILL - 1)
        if c >= 1:
            w_norm(c - 1)
    best, bidx = st['best'], st['bidx']

    rmax = jnp.max(best)
    idx = jnp.min(jnp.where(best == rmax, bidx, S - 1))
    idx = jnp.minimum(idx, S - 1)
    g0 = pl.multiple_of((idx // 16) * 16, 16)
    xs = hn_v[pl.ds(g0, 16), :]
    cp_wg.wait()
    cp_wu.wait()
    cp_wd.wait()
    a = jnp.dot(xs, wg_v[...], preferred_element_type=F32)
    u = jnp.dot(xs, wu_v[...], preferred_element_type=F32)
    a = a.astype(BF16).astype(F32)
    u = u.astype(BF16).astype(F32)
    gu = (a * jax.nn.sigmoid(a) * u).astype(BF16)
    y = jnp.dot(gu, wd_v[...], preferred_element_type=F32)
    rs = jax.nn.sigmoid(jnp.full((1, 1), rmax, F32))
    sel = lax.broadcasted_iota(jnp.int32, (16, D), 0) == (idx - g0)
    base = ob_v[pl.ds(g0, 16), :].astype(F32)
    fx_v[...] = (base + jnp.where(sel, y * rs, 0.0)).astype(BF16)
    for c in range(NO):
        cp_o[c].wait()
    cp_f = pltpu.make_async_copy(fx_v, out_hbm.at[pl.ds(g0, 16)], osem.at[NO])
    cp_f.start()
    cp_f.wait()


@jax.jit
def pallas_sequential_preLN__mha_block__moe_arch_mod__prompt_kernel(
        A_x, A_wqkv, A_wo, B_x, B_w_r, B_w_gate, B_w_up, B_w_down):
    del B_x
    x = A_x.reshape(S, D)
    anyspec = pl.BlockSpec(memory_space=pl.ANY)
    out = pl.pallas_call(
        _kernel,
        out_shape=jax.ShapeDtypeStruct((S, D), BF16),
        in_specs=[anyspec] * 7,
        out_specs=anyspec,
        scratch_shapes=[
            pltpu.VMEM((S, D), BF16), pltpu.VMEM((D, D), BF16), pltpu.VMEM((D, D), BF16),
            pltpu.VMEM((D, D), BF16), pltpu.VMEM((D, D), BF16),
            pltpu.VMEM((D,), BF16), pltpu.VMEM((D, F), BF16), pltpu.VMEM((D, F), BF16),
            pltpu.VMEM((F, D), BF16),
            pltpu.VMEM((S, D), BF16),
            pltpu.VMEM((9, S, 128), BF16), pltpu.VMEM((D, S), BF16), pltpu.VMEM((D, S), F32),
            pltpu.VMEM((2 * S, QB), F32), pltpu.VMEM((D, S), F32), pltpu.VMEM((S, D), F32),
            pltpu.VMEM((S, D), BF16),
            pltpu.VMEM((S, D), BF16), pltpu.VMEM((16, D), BF16),
            pltpu.SemaphoreType.DMA((3,)), pltpu.SemaphoreType.DMA((8,)),
            pltpu.SemaphoreType.DMA((NO + 1,)),
        ],
        compiler_params=pltpu.CompilerParams(vmem_limit_bytes=100 * 1024 * 1024),
        name="seqk",
    )(x, A_wqkv, A_wo, B_w_r, B_w_gate, B_w_up, B_w_down)
    return out.reshape(1, S, D)
```

```python
import numpy as np
import jax
import jax.numpy as jnp
from jax import lax
import jax.experimental.pallas as pl
import jax.experimental.pallas.tpu as pltpu

S, D, H, DH, F = 2048, 640, 32, 20, 1536
QB = 512
C = 128
NCH = S // C
NQ = S // QB
TP = 256
NP = S // TP
TW = 128
NW = S // TW
TO = 256
NO = S // TO
HPB = 2
PEEL = 2
NFILL = 4
EPS = 1e-5
QSCALE = float(DH ** -0.5 * np.log2(np.e))
F32 = jnp.float32
BF16 = jnp.bfloat16
TN = (((0,), (0,)), ((), ()))
NN = (((1,), (0,)), ((), ()))


def _ln(x):
    mu = jnp.mean(x, axis=-1, keepdims=True)
    d = x - mu
    var = jnp.mean(d * d, axis=-1, keepdims=True)
    return d * lax.rsqrt(var + EPS)


def _kernel(x_hbm, wqkv_hbm, wo_hbm, wr_hbm, wg_hbm, wu_hbm, wd_hbm, out_hbm,
            x_v, wq_v, wk_v, wv_v, wo_v, wr_v, wg_v, wu_v, wd_v,
            xn_v, kw_v, qt_v, vt_v, s_v, ot_v, h_v, hn_v, ob_v, fx_v,
            xsem, wsem, osem):
    def xcopy(r0, n, i):
        return pltpu.make_async_copy(x_hbm.at[pl.ds(r0, n)], x_v.at[pl.ds(r0, n)], xsem.at[i])
    cp_x0 = xcopy(0, TP, 0)
    cp_x1 = xcopy(TP, TP, 1)
    cp_x2 = xcopy(2 * TP, S - 2 * TP, 2)
    cp_wq = pltpu.make_async_copy(wqkv_hbm.at[:, pl.ds(0, D)], wq_v, wsem.at[0])
    cp_wk = pltpu.make_async_copy(wqkv_hbm.at[:, pl.ds(D, D)], wk_v, wsem.at[1])
    cp_wv = pltpu.make_async_copy(wqkv_hbm.at[:, pl.ds(2 * D, D)], wv_v, wsem.at[2])
    cp_wo = pltpu.make_async_copy(wo_hbm, wo_v, wsem.at[3])
    cp_wr = pltpu.make_async_copy(wr_hbm, wr_v, wsem.at[4])
    cp_wg = pltpu.make_async_copy(wg_hbm, wg_v, wsem.at[5])
    cp_wu = pltpu.make_async_copy(wu_hbm, wu_v, wsem.at[6])
    cp_wd = pltpu.make_async_copy(wd_hbm, wd_v, wsem.at[7])
    for cp in (cp_x0, cp_wk, cp_x1):
        cp.start()

    def ln1(r0, n):
        xn_v[r0:r0 + n, :] = _ln(x_v[r0:r0 + n, :].astype(F32)).astype(BF16)

    def kproj(c):
        r0 = c * TP
        k = jnp.dot(xn_v[r0:r0 + TP, :], wk_v[...], preferred_element_type=F32).astype(BF16)
        for w in range(5):
            kw_v[w, r0:r0 + TP, :] = k[:, 128 * w:128 * (w + 1)]
        for j in range(4):
            kw_v[5 + j, r0:r0 + TP, :] = k[:, 64 + 128 * j:192 + 128 * j]

    def qproj(c):
        r0 = c * TP
        q = jnp.dot(xn_v[r0:r0 + TP, :], wq_v[...], preferred_element_type=F32)
        qt_v[:, r0:r0 + TP] = (q * QSCALE).astype(BF16).T

    def vproj(c):
        r0 = c * TP
        v = jnp.dot(xn_v[r0:r0 + TP, :], wv_v[...], preferred_element_type=F32)
        vt_v[:, r0:r0 + TP] = v.astype(BF16).T.astype(F32)

    cp_x0.wait()
    cp_wq.start()
    cp_wv.start()
    ln1(0, TP)
    cp_wk.wait()
    cp_x1.wait()
    cp_x2.start()
    kproj(0)
    ln1(TP, TP)
    kproj(1)
    cp_wq.wait()
    cp_wv.wait()
    for cp in (cp_wo, cp_wr, cp_wg, cp_wu, cp_wd):
        cp.start()
    qproj(0)
    vproj(0)
    cp_x2.wait()
    qproj(1)
    ln1(2 * TP, TP // 2)
    vproj(1)
    ln1(2 * TP + TP // 2, TP // 2)
    for c in range(2, NP):
        qproj(c)
        if c + 1 < NP:
            ln1((c + 1) * TP, TP // 2)
        kproj(c)
        if c + 1 < NP:
            ln1((c + 1) * TP + TP // 2, TP // 2)
        vproj(c)

    def head_geom(h):
        f0 = h * DH
        t = f0 // 128
        rem = f0 - t * 128
        strad = rem > 128 - DH
        if isinstance(h, int):
            o = t * 128 + (64 if strad else 0)
            return (5 + t if strad else t), o, f0 - o
        win = jnp.where(strad, 5 + t, t)
        o = t * 128 + jnp.where(strad, 64, 0)
        return win, pl.multiple_of(o, 64), f0 - o

    def getq(h, qb, geom=None):
        win, o, lo = head_geom(h) if geom is None else geom
        qt = qt_v[pl.ds(o, 128), qb * QB:(qb + 1) * QB]
        rows = lax.broadcasted_iota(jnp.int32, (128, QB), 0)
        qt = jnp.where((rows >= lo) & (rows < lo + DH), qt.astype(F32), 0.0).astype(BF16)
        return win, qt

    def stage_a(item, half, j, mx):
        win, qt = item
        s = jnp.dot(kw_v[win, j * C:(j + 1) * C, :], qt, preferred_element_type=F32)
        s_v[half * S + j * C:half * S + (j + 1) * C, :] = s
        mj = jnp.max(s.reshape(C // 8, 8, QB), axis=0)
        return mj if mx is None else jnp.maximum(mx, mj)

    def stage_b(a_h, ones_mask, half, j, m, acc):
        s = s_v[half * S + j * C:half * S + (j + 1) * C, :]
        p = jnp.exp2(s - m).astype(BF16)
        vt = vt_v[pl.ds(a_h, 24), j * C:(j + 1) * C]
        vt = jnp.where(ones_mask, 1.0, vt)
        pv = lax.dot_general(vt, p, NN, preferred_element_type=F32)
        return pv if acc is None else acc + pv

    def red(mx):
        return jnp.max(mx, axis=0, keepdims=True)

    item0 = getq(0, 0)
    mx = None
    for j in range(NCH):
        mx = stage_a(item0, 0, j, mx)
    m0 = red(mx)
    mx1 = stage_a(getq(0, 1), 1, 0, None)

    def heads(h0, nh, carry, last, filler=None):
        m, mxn = carry[:2]
        nit = nh * NQ

        def item(u):
            if last and u >= nit:
                return None
            return getq(h0 + u // NQ, u % NQ)

        if len(carry) > 2:
            win0, o0, lo0 = carry[2:]
            nxt = getq(h0, 1, (win0, pl.multiple_of(o0, 64), lo0))
        else:
            nxt = item(1)
        for hh in range(nh):
            h = h0 + hh
            odd = (hh % 2) == 1
            a_h = h * DH - (hh % 2) * 4
            if not isinstance(a_h, int):
                a_h = pl.multiple_of(a_h, 8)
            lo_v = 4 if odd else 0
            ones_row = 0 if odd else 20
            ones_mask = lax.broadcasted_iota(jnp.int32, (24, C), 0) == ones_row
            row24q = lax.broadcasted_iota(jnp.int32, (24, QB), 0)
            valid = (row24q >= lo_v) & (row24q < lo_v + DH)
            for uu in range(NQ):
                u = hh * NQ + uu
                nxt2 = item(u + 2)
                acc = None
                mx2 = None
                for c in range(NCH):
                    if c + 1 < NCH:
                        if nxt is not None:
                            mxn = stage_a(nxt, (u + 1) % 2, c + 1, mxn)
                    elif nxt2 is not None:
                        mx2 = stage_a(nxt2, u % 2, 0, mx2)
                    acc = stage_b(a_h, ones_mask, u % 2, c, m, acc)
                    if filler is not None:
                        filler(u, c)
                denom = acc[ones_row:ones_row + 1, :]
                o = acc * (1.0 / denom)
                pltpu.store(ot_v.at[pl.ds(a_h, 24), uu * QB:(uu + 1) * QB], o, mask=valid)
                if nxt is not None:
                    m = red(mxn)
                mxn = mx2
                nxt = nxt2
        return m, mxn

    def loop_body(hb, cr):
        m, mxn = heads(hb * HPB, HPB, cr, False)
        return (m, mxn) + tuple(head_geom((hb + 1) * HPB))

    geom0 = tuple(jnp.int32(v) for v in head_geom(0))
    carry = lax.fori_loop(0, (H - PEEL) // HPB, loop_body, (m0, mx1) + geom0)[:2]

    cp_o = [pltpu.make_async_copy(ob_v.at[pl.ds(c * TO, TO)], out_hbm.at[pl.ds(c * TO, TO)], osem.at[c])
            for c in range(NO)]
    st = {}

    def w_proj(c):
        r0 = c * TW
        ot = ot_v[:, r0:r0 + TW].astype(BF16)
        attn = lax.dot_general(ot, wo_v[...], TN, preferred_element_type=F32)
        h_v[r0:r0 + TW, :] = x_v[r0:r0 + TW, :].astype(F32) + attn

    def w_norm(c):
        r0 = c * TW
        h = h_v[r0:r0 + TW, :]
        hn = _ln(h)
        ob_v[r0:r0 + TW, :] = (h + hn).astype(BF16)
        if (r0 + TW) % TO == 0:
            cp_o[r0 // TO].start()
        hn_v[r0:r0 + TW, :] = hn.astype(BF16)
        r = jnp.sum(hn * st['wr'], axis=-1, keepdims=True)
        r3 = r.reshape(TW // 8, 8, 1)
        tok = r0 + lax.broadcasted_iota(jnp.int32, (TW // 8, 8, 1), 0) * 8 \
            + lax.broadcasted_iota(jnp.int32, (TW // 8, 8, 1), 1)
        cmax = jnp.max(r3, axis=0)
        cidx = jnp.min(jnp.where(r3 == cmax[None], tok, S), axis=0)
        if 'best' not in st:
            st['best'], st['bidx'] = cmax, cidx
        else:
            gt = cmax > st['best']
            st['best'] = jnp.where(gt, cmax, st['best'])
            st['bidx'] = jnp.where(gt, cidx, st['bidx'])

    def filler(u, c):
        if u == PEEL * NQ - 1 and c % (NCH // NFILL) == 1:
            w_proj(c // (NCH // NFILL))

    cp_wo.wait()
    cp_wr.wait()
    st['wr'] = wr_v[...].astype(F32).reshape(1, D)
    heads(H - PEEL, PEEL, carry, True, filler)
    for c in range(NW + 1):
        if 1 <= c and c + NFILL - 1 < NW:
            w_proj(c + NFILL - 1)
        if c >= 1:
            w_norm(c - 1)
    best, bidx = st['best'], st['bidx']

    rmax = jnp.max(best)
    idx = jnp.min(jnp.where(best == rmax, bidx, S - 1))
    idx = jnp.minimum(idx, S - 1)
    g0 = pl.multiple_of((idx // 16) * 16, 16)
    xs = hn_v[pl.ds(g0, 16), :]
    cp_wg.wait()
    cp_wu.wait()
    cp_wd.wait()
    a = jnp.dot(xs, wg_v[...], preferred_element_type=F32)
    u = jnp.dot(xs, wu_v[...], preferred_element_type=F32)
    a = a.astype(BF16).astype(F32)
    u = u.astype(BF16).astype(F32)
    gu = (a * jax.nn.sigmoid(a) * u).astype(BF16)
    y = jnp.dot(gu, wd_v[...], preferred_element_type=F32)
    rs = jax.nn.sigmoid(jnp.full((1, 1), rmax, F32))
    sel = lax.broadcasted_iota(jnp.int32, (16, D), 0) == (idx - g0)
    base = ob_v[pl.ds(g0, 16), :].astype(F32)
    fx_v[...] = (base + jnp.where(sel, y * rs, 0.0)).astype(BF16)
    for c in range(NO):
        cp_o[c].wait()
    cp_f = pltpu.make_async_copy(fx_v, out_hbm.at[pl.ds(g0, 16)], osem.at[NO])
    cp_f.start()
    cp_f.wait()


@jax.jit
def pallas_sequential_preLN__mha_block__moe_arch_mod__prompt_kernel(
        A_x, A_wqkv, A_wo, B_x, B_w_r, B_w_gate, B_w_up, B_w_down):
    del B_x
    x = A_x.reshape(S, D)
    anyspec = pl.BlockSpec(memory_space=pl.ANY)
    out = pl.pallas_call(
        _kernel,
        out_shape=jax.ShapeDtypeStruct((S, D), BF16),
        in_specs=[anyspec] * 7,
        out_specs=anyspec,
        scratch_shapes=[
            pltpu.VMEM((S, D), BF16), pltpu.VMEM((D, D), BF16), pltpu.VMEM((D, D), BF16),
            pltpu.VMEM((D, D), BF16), pltpu.VMEM((D, D), BF16),
            pltpu.VMEM((D,), BF16), pltpu.VMEM((D, F), BF16), pltpu.VMEM((D, F), BF16),
            pltpu.VMEM((F, D), BF16),
            pltpu.VMEM((S, D), BF16),
            pltpu.VMEM((9, S, 128), BF16), pltpu.VMEM((D, S), BF16), pltpu.VMEM((D, S), F32),
            pltpu.VMEM((2 * S, QB), F32), pltpu.VMEM((D, S), F32), pltpu.VMEM((S, D), F32),
            pltpu.VMEM((S, D), BF16),
            pltpu.VMEM((S, D), BF16), pltpu.VMEM((16, D), BF16),
            pltpu.SemaphoreType.DMA((3,)), pltpu.SemaphoreType.DMA((8,)),
            pltpu.SemaphoreType.DMA((NO + 1,)),
        ],
        compiler_params=pltpu.CompilerParams(vmem_limit_bytes=100 * 1024 * 1024),
        name="seqk",
    )(x, A_wqkv, A_wo, B_w_r, B_w_gate, B_w_up, B_w_down)
    return out.reshape(1, S, D)
```
